```python
import os as _os
_os.environ.setdefault("JAX_PLATFORMS", "cpu")
import jax
import jax.numpy as jnp

def _softmax(x, axis=-1):
    return jax.nn.softmax(x, axis=axis)
def _gelu(x):
    return jax.nn.gelu(x, approximate=True)
def _silu(x):
    return jax.nn.silu(x)
def _sigmoid(x):
    return jax.nn.sigmoid(x)
def _layernorm(x, axis=-1, eps=1e-5):
    m = jnp.mean(x, axis=axis, keepdims=True)
    v = jnp.var(x, axis=axis, keepdims=True)
    return (x - m) / jnp.sqrt(v + eps)
def _scatter_add(tgt, idx, src, axis=0):
    return tgt.at[idx].add(src)
def _segment_sum(src, seg, n):
    return jax.ops.segment_sum(src, seg, n)
class _Rng:
    def __init__(self, key):
        self._k = key
    def _next(self):
        self._k, sub = jax.random.split(self._k)
        return sub
    def normal(self, shape):
        return jax.random.normal(self._next(), shape, dtype=jnp.bfloat16)
    def randint(self, lo, hi, shape):
        return jax.random.randint(self._next(), shape, lo, hi, dtype=jnp.int32)
    def uniform(self, shape, lo=0.0, hi=1.0):
        return jax.random.uniform(self._next(), shape, jnp.bfloat16, lo, hi)
    def permutation(self, n):
        return jax.random.permutation(self._next(), n)


kernel_name = 'parallel_sum__spectral_gfnet__glu_gated_swiglu__prompt'

def setup_inputs():
    _rng = _Rng(jax.random.key(int.from_bytes(__import__("os").urandom(4), "little")))
    _w = (lambda a: (lambda t: t.astype(jnp.bfloat16) if jnp.issubdtype(t.dtype, jnp.floating) else t)(jnp.asarray(a)))
    def _A_setup():
        B, S, D = 1, 2048, 512
        Df = D // 2 + 1
        return {
            "x": _w((lambda *s: _rng.normal(s) * 0.05)(B, S, D)),
            "w_r": _w((lambda *s: _rng.normal(s) * 0.2)(S, Df) * 0.02),
            "w_i": _w((lambda *s: _rng.normal(s) * 0.2)(S, Df) * 0.02),
        }
    _A_in = _A_setup()

    def _B_setup():
        B, S, D, F = 1, 2048, 512, 1376
        return {
            "x": _w((lambda *s: _rng.normal(s) * 0.05)(B, S, D)),
            "w1": _w((lambda *s: _rng.normal(s) * 0.05)(D, F) * (2.0 / D) ** 0.5),
            "w3": _w((lambda *s: _rng.normal(s) * 0.05)(D, F) * (2.0 / D) ** 0.5),
            "w2": _w((lambda *s: _rng.normal(s) * 0.05)(F, D) * (2.0 / F) ** 0.5),
        }
    _B_in = _B_setup()

    return {
        "A_x": _A_in["x"],
        "A_w_r": _A_in["w_r"],
        "A_w_i": _A_in["w_i"],
        "B_x": _B_in["x"],
        "B_w1": _B_in["w1"],
        "B_w3": _B_in["w3"],
        "B_w2": _B_in["w2"],
    }

def reference(A_x, A_w_r, A_w_i, B_x, B_w1, B_w3, B_w2):
    def _A_ref(x, w_r, w_i):
        B, S, D = x.shape
        X = (lambda x, axes=(-2,-1): jnp.fft.rfft2(x.astype(jnp.float32), axes=axes))(x, axes=(-2, -1))
        W = w_r + 1j * w_i
        X = X * W
        y = (lambda x, s, axes=(-2,-1): jnp.fft.irfft2(x, s=s, axes=axes).astype(jnp.bfloat16))(X, (S, D), axes=(-2, -1))
        return y

    def _B_ref(x, w1, w3, w2):
        gate = jnp.einsum("bsd,df->bsf", x, w1)
        up = jnp.einsum("bsd,df->bsf", x, w3)
        h = _silu(gate) * up
        out = jnp.einsum("bsf,fd->bsd", h, w2)
        return out

    x = A_x
    xn = _layernorm(x, axis=-1)
    return x + _A_ref(xn, A_w_r, A_w_i) + _B_ref(xn, B_w1, B_w3, B_w2)
```

```python
import math

import jax
import jax.numpy as jnp
import numpy as np
import jax.experimental.pallas as pl
import jax.experimental.pallas.tpu as pltpu

S, D, F = 2048, 512, 1376
R = 16
M = S // R
H = D // 2
BM = 256
NB = S // BM
BF16 = jnp.bfloat16
F32 = jnp.float32


def _consts():
    d = np.arange(D)[:, None]
    k = np.arange(H)[None, :]
    ang = 2 * np.pi * ((d * k) % D) / D
    fd = np.concatenate([np.cos(ang), -np.sin(ang)], axis=1)
    fd[:, H] = (-1.0) ** np.arange(D)
    gd = 2.0 * fd.T / D
    gd[0] /= 2
    gd[H] /= 2
    b = np.arange(M)[None, :]
    kb = np.arange(M)[:, None]
    fs = []
    for ka in range(R):
        a = 2 * np.pi * ((b * (ka + R * kb)) % S) / S
        fr, fi = np.cos(a), -np.sin(a)
        fs.append(np.block([[fr, -fi], [fi, fr]]))
    fs = np.stack(fs)
    gs = np.transpose(fs, (0, 2, 1)) / S
    j = np.zeros((2, M, M))
    i = np.arange(M)
    j[0, i, (M - i) % M] = 1
    j[1, i, M - 1 - i] = 1
    c = lambda t: np.asarray(t, np.float32).astype(BF16)
    return c(fd), c(gd), c(fs), c(gs), c(j)


def _bf4(x, sign):
    (ar, ai), (br, bi), (cr, ci), (dr, di) = x
    sr, si, tr, ti = ar + cr, ai + ci, ar - cr, ai - ci
    ur, ui, vr, vi = br + dr, bi + di, br - dr, bi - di
    p = (tr + vi, ti - vr)
    q = (tr - vi, ti + vr)
    if sign > 0:
        p, q = q, p
    return [(sr + ur, si + ui), p, (sr - ur, si - ui), q]


def _tw(z, e, sign):
    r, i = z
    e = e % 16
    if e == 0:
        return z
    if e == 4:
        return (-i, r) if sign > 0 else (i, -r)
    c = math.cos(2 * math.pi * e / 16)
    s = sign * math.sin(2 * math.pi * e / 16)
    if e in (2, 6):
        if c * s > 0:
            return ((r - i) * c, (r + i) * c)
        return ((r + i) * c, (i - r) * c)
    return (r * c - i * s, i * c + r * s)


def _fft16(x, sign):
    t = [_bf4([x[4 * n1 + n2] for n1 in range(4)], sign) for n2 in range(4)]
    out = [None] * 16
    for k1 in range(4):
        o = _bf4([_tw(t[n2][k1], n2 * k1, sign) for n2 in range(4)], sign)
        for k2 in range(4):
            out[k1 + 4 * k2] = o[k2]
    return out


def _dot(a, b):
    return jnp.dot(a, b, preferred_element_type=F32)


def _kernel(x_h, wr_h, wi_h, w1_h, w3_h, w2_h, fd_h, gd_h, fs_h, gs_h, j_h, o_h,
            x_v, wr_v, wi_v, w1_v, w3_v, w2_v, fd_v, gd_v, fs_v, gs_v, j_v,
            xn_v, z_v, acc_v, o_v, wu_v, sem, osem):
    cp = lambda s, d, i: pltpu.make_async_copy(s, d, sem.at[i])
    c_fd = cp(fd_h, fd_v, 0)
    c_x = [cp(x_h.at[pl.ds(i * BM, BM)], x_v.at[pl.ds(i * BM, BM)], 16 + i) for i in range(NB)]
    rest = [cp(w1_h, w1_v, 1), cp(w3_h, w3_v, 2), cp(w2_h, w2_v, 3), cp(fs_h, fs_v, 4),
            cp(wr_h, wr_v, 5), cp(wi_h, wi_v, 6), cp(j_h, j_v, 7), cp(gs_h, gs_v, 8),
            cp(gd_h, gd_v, 9)]
    c_x[0].start()
    c_fd.start()
    for c in c_x[1:] + rest:
        c.start()

    c_fd.wait()
    for i in range(NB):
        c_x[i].wait()
        rows = pl.ds(i * BM, BM)
        x = x_v[rows, :].astype(F32)
        xc = x - jnp.mean(x, axis=-1, keepdims=True)
        v = jnp.mean(xc * xc, axis=-1, keepdims=True)
        xn = (xc * jax.lax.rsqrt(v + 1e-5)).astype(BF16)
        xn_v[rows, :] = xn
        z_v[rows, :] = _dot(xn, fd_v[...])

    def ffn(i):
        rows = pl.ds(pl.multiple_of(i * BM, BM), BM)
        xn = xn_v[rows, :]
        g = _dot(xn, w1_v[...])
        u = _dot(xn, w3_v[...])
        h = (g * jax.nn.sigmoid(g) * u).astype(BF16)
        acc_v[rows, :] = _dot(h, w2_v[...]) + x_v[rows, :].astype(F32)

    def butterflies(r0, n, sign):
        for r in range(n // 8):
            for c in range(H // 128):
                sl = lambda a, im: (pl.ds(a * M + r0 + 8 * r, 8), pl.ds(im * H + c * 128, 128))
                o = _fft16([(z_v[sl(a, 0)], z_v[sl(a, 1)]) for a in range(R)], sign)
                for a in range(R):
                    z_v[sl(a, 0)] = o[a][0]
                    z_v[sl(a, 1)] = o[a][1]

    def pack_w(i):
        for t in range(4):
            r = i * 1024 + t * 256
            src = pl.ds(pl.multiple_of(r, 256), 256)
            dst = pl.ds(pl.multiple_of(r // 2, 128), 128)
            for n, ref in enumerate((wr_v, wi_v)):
                for c in range(2):
                    wu_v[3 * n + c, dst, :] = pltpu.bitcast(ref[src, pl.ds(c * 128, 128)], jnp.uint32)
                w = jnp.broadcast_to(ref[src, pl.ds(H, 1)].astype(F32), (256, 128)).astype(BF16)
                wu_v[3 * n + 2, dst, :] = pltpu.bitcast(w, jnp.uint32)

    def load_w(n, ka):
        u = wu_v[n, pl.ds(ka // 2, M, stride=R // 2), :]
        u = (u & jnp.uint32(0xFFFF0000)) if ka % 2 else (u << 16)
        return jax.lax.bitcast_convert_type(u, F32)

    lane0 = jax.lax.broadcasted_iota(jnp.int32, (M, 128), 1) == 0

    def spectral(kas):
        jm = j_v[0] if kas[0] == 0 else j_v[1]
        rev = lambda t: _dot(jm, t.astype(BF16))
        p, q, rm = {}, {}, {}
        for ka in kas:
            rows = pl.ds(ka * M, M)
            u = jnp.concatenate([z_v[rows, pl.ds(0, H)], z_v[rows, pl.ds(H, H)]], axis=0)
            t = _dot(fs_v[ka], u.astype(BF16))
            p[ka] = (t[:M], t[M:])
        for ka in kas:
            pr, pi = p[ka]
            ur, ui = load_w(0, ka), load_w(3, ka)
            wr = jnp.concatenate([ur, load_w(1, ka)], axis=1)
            wi = jnp.concatenate([ui, load_w(4, ka)], axis=1)
            q[ka] = (pr * wr - pi * wi, pr * wi + pi * wr)
            vr, vi = load_w(2, ka), load_w(5, ka)
            nr, ni = p[(R - ka) % R]
            nr, ni = rev(nr[:, :128]), rev(ni[:, :128])
            pr, pi = pr[:, :128], pi[:, :128]
            ar, ai, br, bi = pr + nr, pi - ni, pr - nr, pi + ni
            er, ei = ar * ur - ai * ui, ar * ui + ai * ur
            fr, fi = br * vr - bi * vi, br * vi + bi * vr
            rm[ka] = (er + fr, ei + fi, er - fr, ei - fi)
        for ka in kas:
            qr, qi = q[ka]
            m = rm[(R - ka) % R]
            q0r = jnp.where(lane0, 0.25 * (rm[ka][0] + rev(m[2])), qr[:, :128])
            q0i = jnp.where(lane0, 0.25 * (rm[ka][1] - rev(m[3])), qi[:, :128])
            qq = jnp.concatenate([jnp.concatenate([q0r, qr[:, 128:]], axis=1),
                                  jnp.concatenate([q0i, qi[:, 128:]], axis=1)], axis=0)
            t = _dot(gs_v[ka], qq.astype(BF16))
            rows = pl.ds(ka * M, M)
            z_v[rows, pl.ds(0, H)] = t[:M]
            z_v[rows, pl.ds(H, H)] = t[M:]

    for c in rest[:3] + rest[4:6]:
        c.wait()

    def fwd(i, _):
        ffn(i)
        pack_w(i)
        butterflies(pl.multiple_of(i * 64, 64), 64, -1)
    jax.lax.fori_loop(0, 2, fwd, None)

    for c in [rest[3]] + rest[6:8]:
        c.wait()
    groups = [[0], [8]] + [[a, R - a] for a in range(1, 8)]
    for i, gr in enumerate([groups[0:3], groups[3:5], groups[5:7], groups[7:9]]):
        ffn(2 + i)
        for kas in gr:
            spectral(kas)

    def inv(i, _):
        ffn(i + 6)
        butterflies(pl.multiple_of(i * 64, 64), 64, 1)
    jax.lax.fori_loop(0, 2, inv, None)

    rest[8].wait()
    outs = []
    for i in range(NB):
        rows = pl.ds(i * BM, BM)
        y = _dot(z_v[rows, :].astype(BF16), gd_v[...])
        o_v[rows, :] = (acc_v[rows, :] + y).astype(BF16)
        c = pltpu.make_async_copy(o_v.at[rows], o_h.at[rows], osem.at[i])
        c.start()
        outs.append(c)
    for c in outs:
        c.wait()


@jax.jit
def pallas_parallel_sum__spectral_gfnet__glu_gated_swiglu__prompt_kernel(
    A_x, A_w_r, A_w_i, B_x, B_w1, B_w3, B_w2,
):
    del B_x
    args = (A_x.reshape(S, D), A_w_r, A_w_i, B_w1, B_w3, B_w2) + _consts()
    out = pl.pallas_call(
        _kernel,
        out_shape=jax.ShapeDtypeStruct((S, D), BF16),
        in_specs=[pl.BlockSpec(memory_space=pl.ANY)] * len(args),
        out_specs=pl.BlockSpec(memory_space=pl.ANY),
        scratch_shapes=[pltpu.VMEM(a.shape, a.dtype) for a in args] + [
            pltpu.VMEM((S, D), BF16), pltpu.VMEM((S, D), F32), pltpu.VMEM((S, D), F32),
            pltpu.VMEM((S, D), BF16), pltpu.VMEM((6, S // 2, 128), jnp.uint32),
            pltpu.SemaphoreType.DMA((16 + NB,)), pltpu.SemaphoreType.DMA((NB,))],
        compiler_params=pltpu.CompilerParams(vmem_limit_bytes=64 * 1024 * 1024),
    )(*args)
    return out.reshape(1, S, D)
```

```python
import math

import jax
import jax.numpy as jnp
import numpy as np
import jax.experimental.pallas as pl
import jax.experimental.pallas.tpu as pltpu

S, D, F = 2048, 512, 1376
R = 16
M = S // R
H = D // 2
BM = 256
NB = S // BM
BF16 = jnp.bfloat16
F32 = jnp.float32


def _consts():
    d = np.arange(D)[:, None]
    k = np.arange(H)[None, :]
    ang = 2 * np.pi * ((d * k) % D) / D
    fd = np.concatenate([np.cos(ang), -np.sin(ang)], axis=1)
    fd[:, H] = (-1.0) ** np.arange(D)
    gd = 2.0 * fd.T / D
    gd[0] /= 2
    gd[H] /= 2
    cols = [np.concatenate([np.arange(p, H, 2), H + np.arange(p, H, 2)]) for p in (0, 1)]
    fd = np.stack([fd[:H][:, c] for c in cols])
    gd = np.stack([gd[c][:, :H] for c in cols])
    b = np.arange(M)[None, :]
    kb = np.arange(M)[:, None]
    fs = []
    for ka in range(R):
        a = 2 * np.pi * ((b * (ka + R * kb)) % S) / S
        fr, fi = np.cos(a), -np.sin(a)
        fs.append(np.block([[fr, -fi], [fi, fr]]))
    fs = np.stack(fs)
    gs = np.transpose(fs, (0, 2, 1)) / S
    j = np.zeros((2, M, M))
    i = np.arange(M)
    j[0, i, (M - i) % M] = 1
    j[1, i, M - 1 - i] = 1
    c = lambda t: np.asarray(t, np.float32).astype(BF16)
    return c(fd), c(gd), c(fs), c(gs), c(j)


def _bf4(x, sign):
    (ar, ai), (br, bi), (cr, ci), (dr, di) = x
    sr, si, tr, ti = ar + cr, ai + ci, ar - cr, ai - ci
    ur, ui, vr, vi = br + dr, bi + di, br - dr, bi - di
    p = (tr + vi, ti - vr)
    q = (tr - vi, ti + vr)
    if sign > 0:
        p, q = q, p
    return [(sr + ur, si + ui), p, (sr - ur, si - ui), q]


def _tw(z, e, sign):
    r, i = z
    e = e % 16
    if e == 0:
        return z
    if e == 4:
        return (-i, r) if sign > 0 else (i, -r)
    c = math.cos(2 * math.pi * e / 16)
    s = sign * math.sin(2 * math.pi * e / 16)
    if e in (2, 6):
        if c * s > 0:
            return ((r - i) * c, (r + i) * c)
        return ((r + i) * c, (i - r) * c)
    return (r * c - i * s, i * c + r * s)


def _fft16(x, sign):
    t = [_bf4([x[4 * n1 + n2] for n1 in range(4)], sign) for n2 in range(4)]
    out = [None] * 16
    for k1 in range(4):
        o = _bf4([_tw(t[n2][k1], n2 * k1, sign) for n2 in range(4)], sign)
        for k2 in range(4):
            out[k1 + 4 * k2] = o[k2]
    return out


def _dot(a, b):
    return jnp.dot(a, b, preferred_element_type=F32)


def _dot_t(a, b):
    return jax.lax.dot_general(a, b, (((1,), (1,)), ((), ())), preferred_element_type=F32)


def _kernel(x_h, wr_h, wi_h, w1_h, w3_h, w2_h, fd_h, gd_h, fs_h, gs_h, j_h, o_h,
            x_v, wr_v, wi_v, w1_v, w3_v, w2_v, fd_v, gd_v, fs_v, gs_v, j_v,
            xn_v, z_v, acc_v, o_v, wu_v, sem, osem):
    cp = lambda s, d, i: pltpu.make_async_copy(s, d, sem.at[i])
    c_fd = cp(fd_h, fd_v, 0)
    c_x = [cp(x_h.at[pl.ds(i * BM, BM)], x_v.at[pl.ds(i * BM, BM)], 16 + i) for i in range(NB)]
    rest = [cp(w1_h, w1_v, 1), cp(w3_h, w3_v, 2), cp(w2_h, w2_v, 3), cp(fs_h, fs_v, 4),
            cp(wr_h, wr_v, 5), cp(wi_h, wi_v, 6), cp(j_h, j_v, 7), cp(gs_h, gs_v, 8),
            cp(gd_h, gd_v, 9)]
    c_x[0].start()
    c_fd.start()
    for c in c_x[1:] + rest:
        c.start()

    c_fd.wait()
    for i in range(NB):
        c_x[i].wait()
        rows = pl.ds(i * BM, BM)
        x = x_v[rows, :].astype(F32)
        xc = x - jnp.mean(x, axis=-1, keepdims=True)
        v = jnp.mean(xc * xc, axis=-1, keepdims=True)
        xn = (xc * jax.lax.rsqrt(v + 1e-5)).astype(BF16)
        xn_v[rows, :] = xn
        lo, hi = xn[:, :H].astype(F32), xn[:, H:].astype(F32)
        for p, t in enumerate((lo + hi, lo - hi)):
            t = _dot(t.astype(BF16), fd_v[p])
            z_v[rows, pl.ds(p * 128, 128)] = t[:, :128]
            z_v[rows, pl.ds(H + p * 128, 128)] = t[:, 128:]

    def ffn(i):
        rows = pl.ds(pl.multiple_of(i * BM, BM), BM)
        xn = xn_v[rows, :]
        g = _dot_t(xn, w1_v[...])
        u = _dot_t(xn, w3_v[...])
        h = (g * jax.nn.sigmoid(g) * u).astype(BF16)
        acc_v[rows, :] = _dot(h, w2_v[...]) + x_v[rows, :].astype(F32)

    def butterflies(r0, n, sign):
        for r in range(n // 8):
            for c in range(H // 128):
                sl = lambda a, im: (pl.ds(a * M + r0 + 8 * r, 8), pl.ds(im * H + c * 128, 128))
                o = _fft16([(z_v[sl(a, 0)], z_v[sl(a, 1)]) for a in range(R)], sign)
                for a in range(R):
                    z_v[sl(a, 0)] = o[a][0]
                    z_v[sl(a, 1)] = o[a][1]

    def pack_w(i):
        for t in range(4):
            sl = pl.ds(pl.multiple_of(i * 1024 + t * 256, 256), 256)
            for n, ref in enumerate((wr_v, wi_v)):
                wu_v[n, sl, :] = pltpu.bitcast(ref[pl.ds(0, H), sl], F32).T
                wu_v[2 + n, sl, :] = jnp.broadcast_to(ref[pl.ds(H, 1), sl].astype(F32), (128, 256)).T

    def load_w(n, ka):
        w = wu_v[n, pl.ds(ka, M, stride=R), :]
        if n >= 2:
            return w
        u = jax.lax.bitcast_convert_type(w, jnp.uint32)
        return (jax.lax.bitcast_convert_type(u << 16, F32),
                jax.lax.bitcast_convert_type(u & jnp.uint32(0xFFFF0000), F32))

    lane0 = jax.lax.broadcasted_iota(jnp.int32, (M, 128), 1) == 0

    def spectral(kas):
        jm = j_v[0] if kas[0] == 0 else j_v[1]
        rev = lambda t: _dot(jm, t.astype(BF16))
        p, q, rm = {}, {}, {}
        for ka in kas:
            rows = pl.ds(ka * M, M)
            u = jnp.concatenate([z_v[rows, pl.ds(0, H)], z_v[rows, pl.ds(H, H)]], axis=0)
            t = _dot(fs_v[ka], u.astype(BF16))
            p[ka] = (t[:M], t[M:])
        for ka in kas:
            pr, pi = p[ka]
            (ur, ur1), (ui, ui1) = load_w(0, ka), load_w(1, ka)
            wr = jnp.concatenate([ur, ur1], axis=1)
            wi = jnp.concatenate([ui, ui1], axis=1)
            q[ka] = (pr * wr - pi * wi, pr * wi + pi * wr)
            vr, vi = load_w(2, ka), load_w(3, ka)
            nr, ni = p[(R - ka) % R]
            nr, ni = rev(nr[:, :128]), rev(ni[:, :128])
            pr, pi = pr[:, :128], pi[:, :128]
            ar, ai, br, bi = pr + nr, pi - ni, pr - nr, pi + ni
            er, ei = ar * ur - ai * ui, ar * ui + ai * ur
            fr, fi = br * vr - bi * vi, br * vi + bi * vr
            rm[ka] = (er + fr, ei + fi, er - fr, ei - fi)
        for ka in kas:
            qr, qi = q[ka]
            m = rm[(R - ka) % R]
            q0r = jnp.where(lane0, 0.25 * (rm[ka][0] + rev(m[2])), qr[:, :128])
            q0i = jnp.where(lane0, 0.25 * (rm[ka][1] - rev(m[3])), qi[:, :128])
            qq = jnp.concatenate([jnp.concatenate([q0r, qr[:, 128:]], axis=1),
                                  jnp.concatenate([q0i, qi[:, 128:]], axis=1)], axis=0)
            t = _dot(gs_v[ka], qq.astype(BF16))
            rows = pl.ds(ka * M, M)
            z_v[rows, pl.ds(0, H)] = t[:M]
            z_v[rows, pl.ds(H, H)] = t[M:]

    for c in rest[:3] + rest[4:6]:
        c.wait()

    def fwd(i, _):
        ffn(i)
        pack_w(i)
        butterflies(pl.multiple_of(i * 64, 64), 64, -1)
    jax.lax.fori_loop(0, 2, fwd, None)

    for c in [rest[3]] + rest[6:8]:
        c.wait()
    groups = [[0], [8]] + [[a, R - a] for a in range(1, 8)]
    for i, gr in enumerate([groups[0:3], groups[3:5], groups[5:7], groups[7:9]]):
        ffn(2 + i)
        for kas in gr:
            spectral(kas)

    def inv(i, _):
        ffn(i + 6)
        butterflies(pl.multiple_of(i * 64, 64), 64, 1)
    jax.lax.fori_loop(0, 2, inv, None)

    rest[8].wait()
    outs = []
    for i in range(NB):
        rows = pl.ds(i * BM, BM)
        ye, yo = [_dot(jnp.concatenate([z_v[rows, pl.ds(p * 128, 128)], z_v[rows, pl.ds(H + p * 128, 128)]],
                                       axis=1).astype(BF16), gd_v[p]) for p in (0, 1)]
        y = jnp.concatenate([ye + yo, ye - yo], axis=1)
        o_v[rows, :] = (acc_v[rows, :] + y).astype(BF16)
        c = pltpu.make_async_copy(o_v.at[rows], o_h.at[rows], osem.at[i])
        c.start()
        outs.append(c)
    for c in outs:
        c.wait()


@jax.jit
def pallas_parallel_sum__spectral_gfnet__glu_gated_swiglu__prompt_kernel(
    A_x, A_w_r, A_w_i, B_x, B_w1, B_w3, B_w2,
):
    del B_x
    args = (A_x.reshape(S, D), A_w_r.T, A_w_i.T, B_w1.T, B_w3.T, B_w2) + _consts()
    out = pl.pallas_call(
        _kernel,
        out_shape=jax.ShapeDtypeStruct((S, D), BF16),
        in_specs=[pl.BlockSpec(memory_space=pltpu.MemorySpace.HBM)] * len(args),
        out_specs=pl.BlockSpec(memory_space=pl.ANY),
        scratch_shapes=[pltpu.VMEM(a.shape, a.dtype) for a in args] + [
            pltpu.VMEM((S, D), BF16), pltpu.VMEM((S, D), F32), pltpu.VMEM((S, D), F32),
            pltpu.VMEM((S, D), BF16), pltpu.VMEM((4, S, 128), F32),
            pltpu.SemaphoreType.DMA((16 + NB,)), pltpu.SemaphoreType.DMA((NB,))],
        compiler_params=pltpu.CompilerParams(vmem_limit_bytes=64 * 1024 * 1024),
    )(*args)
    return out.reshape(1, S, D)
```

```python
import math

import jax
import jax.numpy as jnp
import numpy as np
import jax.experimental.pallas as pl
import jax.experimental.pallas.tpu as pltpu

S, D, F = 2048, 512, 1376
R = 16
M = S // R
H = D // 2
BM = 256
NB = S // BM
BF16 = jnp.bfloat16
F32 = jnp.float32


def _consts():
    d = np.arange(D)[:, None]
    k = np.arange(H)[None, :]
    ang = 2 * np.pi * ((d * k) % D) / D
    fd = np.concatenate([np.cos(ang), -np.sin(ang)], axis=1)
    fd[:, H] = (-1.0) ** np.arange(D)
    gd = 2.0 * fd.T / D
    gd[0] /= 2
    gd[H] /= 2
    cols = [np.concatenate([np.arange(p, H, 2), H + np.arange(p, H, 2)]) for p in (0, 1)]
    fd = np.stack([fd[:H][:, c] for c in cols])
    gd = np.stack([gd[c][:, :H] for c in cols])
    b = np.arange(M)[None, :]
    kb = np.arange(M)[:, None]
    fs = []
    for ka in range(R):
        a = 2 * np.pi * ((b * (ka + R * kb)) % S) / S
        fr, fi = np.cos(a), -np.sin(a)
        fs.append(np.block([[fr, -fi], [fi, fr]]))
    fs = np.stack(fs)
    gs = np.transpose(fs, (0, 2, 1)) / S
    j = np.zeros((2, M, M))
    i = np.arange(M)
    j[0, i, (M - i) % M] = 1
    j[1, i, M - 1 - i] = 1
    c = lambda t: np.asarray(t, np.float32).astype(BF16)
    return c(fd), c(gd), c(fs), c(gs), c(j)


def _bf4(x, sign):
    (ar, ai), (br, bi), (cr, ci), (dr, di) = x
    sr, si, tr, ti = ar + cr, ai + ci, ar - cr, ai - ci
    ur, ui, vr, vi = br + dr, bi + di, br - dr, bi - di
    p = (tr + vi, ti - vr)
    q = (tr - vi, ti + vr)
    if sign > 0:
        p, q = q, p
    return [(sr + ur, si + ui), p, (sr - ur, si - ui), q]


def _tw(z, e, sign):
    r, i = z
    e = e % 16
    if e == 0:
        return z
    if e == 4:
        return (-i, r) if sign > 0 else (i, -r)
    c = math.cos(2 * math.pi * e / 16)
    s = sign * math.sin(2 * math.pi * e / 16)
    if e in (2, 6):
        if c * s > 0:
            return ((r - i) * c, (r + i) * c)
        return ((r + i) * c, (i - r) * c)
    return (r * c - i * s, i * c + r * s)


def _fft16(x, sign):
    t = [_bf4([x[4 * n1 + n2] for n1 in range(4)], sign) for n2 in range(4)]
    out = [None] * 16
    for k1 in range(4):
        o = _bf4([_tw(t[n2][k1], n2 * k1, sign) for n2 in range(4)], sign)
        for k2 in range(4):
            out[k1 + 4 * k2] = o[k2]
    return out


def _dot(a, b):
    return jnp.dot(a, b, preferred_element_type=F32)


def _dot_t(a, b):
    return jax.lax.dot_general(a, b, (((1,), (1,)), ((), ())), preferred_element_type=F32)


def _kernel(x_h, wr_h, wi_h, w1_h, w3_h, w2_h, fd_h, gd_h, fs_h, gs_h, j_h, o_h,
            x_v, wr_v, wi_v, w1_v, w3_v, w2_v, fd_v, gd_v, fs_v, gs_v, j_v,
            xn_v, z_v, acc_v, o_v, wu_v, sem, osem):
    cp = lambda s, d, i: pltpu.make_async_copy(s, d, sem.at[i])
    c_fd = cp(fd_h, fd_v, 0)
    c_x = [cp(x_h.at[pl.ds(i * BM, BM)], x_v.at[pl.ds(i * BM, BM)], 16 + i) for i in range(NB)]
    rest = [cp(w1_h, w1_v, 1), cp(w3_h, w3_v, 2), cp(w2_h, w2_v, 3), cp(fs_h, fs_v, 4),
            cp(wr_h, wr_v, 5), cp(wi_h, wi_v, 6), cp(j_h, j_v, 7), cp(gs_h, gs_v, 8),
            cp(gd_h, gd_v, 9)]
    c_x[0].start()
    c_fd.start()
    for c in c_x[1:3] + rest[:1]:
        c.start()

    c_fd.wait()
    for i in range(NB):
        c_x[i].wait()
        if i + 3 < NB:
            c_x[i + 3].start()
        if i == 4:
            rest[1].start()
        if i == 6:
            rest[2].start()
        rows = pl.ds(i * BM, BM)
        x = x_v[rows, :].astype(F32)
        xc = x - jnp.mean(x, axis=-1, keepdims=True)
        v = jnp.mean(xc * xc, axis=-1, keepdims=True)
        xn = (xc * jax.lax.rsqrt(v + 1e-5)).astype(BF16)
        xn_v[rows, :] = xn
        lo, hi = xn[:, :H].astype(F32), xn[:, H:].astype(F32)
        for p, t in enumerate((lo + hi, lo - hi)):
            t = _dot(t.astype(BF16), fd_v[p])
            z_v[rows, pl.ds(p * 128, 128)] = t[:, :128]
            z_v[rows, pl.ds(H + p * 128, 128)] = t[:, 128:]

    def ffn(i):
        rows = pl.ds(i * BM, BM)
        xn = xn_v[rows, :]
        g = _dot_t(xn, w1_v[...])
        u = _dot_t(xn, w3_v[...])
        h = (g * jax.nn.sigmoid(g) * u).astype(BF16)
        acc_v[rows, :] = _dot(h, w2_v[...]) + x_v[rows, :].astype(F32)

    def butterflies(r0, n, sign):
        for r in range(n // 8):
            for c in range(H // 128):
                sl = lambda a, im: (pl.ds(a * M + r0 + 8 * r, 8), pl.ds(im * H + c * 128, 128))
                o = _fft16([(z_v[sl(a, 0)], z_v[sl(a, 1)]) for a in range(R)], sign)
                for a in range(R):
                    z_v[sl(a, 0)] = o[a][0]
                    z_v[sl(a, 1)] = o[a][1]

    def pack_w(i):
        for t in range(4):
            sl = pl.ds(i * 1024 + t * 256, 256)
            for n, ref in enumerate((wr_v, wi_v)):
                wu_v[n, sl, :] = pltpu.bitcast(ref[pl.ds(0, H), sl], F32).T
                wu_v[2 + n, sl, :] = jnp.broadcast_to(ref[pl.ds(H, 1), sl].astype(F32), (128, 256)).T

    def load_w(n, ka):
        w = wu_v[n, pl.ds(ka, M, stride=R), :]
        if n >= 2:
            return w
        u = jax.lax.bitcast_convert_type(w, jnp.uint32)
        return (jax.lax.bitcast_convert_type(u << 16, F32),
                jax.lax.bitcast_convert_type(u & jnp.uint32(0xFFFF0000), F32))

    lane0 = jax.lax.broadcasted_iota(jnp.int32, (M, 128), 1) == 0

    def spectral(kas):
        jm = j_v[0] if kas[0] == 0 else j_v[1]
        rev = lambda t: _dot(jm, t.astype(BF16))
        p, q, rm = {}, {}, {}
        for ka in kas:
            rows = pl.ds(ka * M, M)
            u = jnp.concatenate([z_v[rows, pl.ds(0, H)], z_v[rows, pl.ds(H, H)]], axis=0)
            t = _dot(fs_v[ka], u.astype(BF16))
            p[ka] = (t[:M], t[M:])
        for ka in kas:
            pr, pi = p[ka]
            (ur, ur1), (ui, ui1) = load_w(0, ka), load_w(1, ka)
            wr = jnp.concatenate([ur, ur1], axis=1)
            wi = jnp.concatenate([ui, ui1], axis=1)
            q[ka] = (pr * wr - pi * wi, pr * wi + pi * wr)
            vr, vi = load_w(2, ka), load_w(3, ka)
            nr, ni = p[(R - ka) % R]
            nr, ni = rev(nr[:, :128]), rev(ni[:, :128])
            pr, pi = pr[:, :128], pi[:, :128]
            ar, ai, br, bi = pr + nr, pi - ni, pr - nr, pi + ni
            er, ei = ar * ur - ai * ui, ar * ui + ai * ur
            fr, fi = br * vr - bi * vi, br * vi + bi * vr
            rm[ka] = (er + fr, ei + fi, er - fr, ei - fi)
        for ka in kas:
            qr, qi = q[ka]
            m = rm[(R - ka) % R]
            q0r = jnp.where(lane0, 0.25 * (rm[ka][0] + rev(m[2])), qr[:, :128])
            q0i = jnp.where(lane0, 0.25 * (rm[ka][1] - rev(m[3])), qi[:, :128])
            qq = jnp.concatenate([jnp.concatenate([q0r, qr[:, 128:]], axis=1),
                                  jnp.concatenate([q0i, qi[:, 128:]], axis=1)], axis=0)
            t = _dot(gs_v[ka], qq.astype(BF16))
            rows = pl.ds(ka * M, M)
            z_v[rows, pl.ds(0, H)] = t[:M]
            z_v[rows, pl.ds(H, H)] = t[M:]

    for c in rest[3:]:
        c.start()
    for c in rest[:3]:
        c.wait()
    ffn(0)
    butterflies(0, 64, -1)
    for c in rest[3:8]:
        c.wait()
    ffn(1)
    butterflies(64, 64, -1)
    pack_w(0)
    pack_w(1)
    groups = [[0], [8]] + [[a, R - a] for a in range(1, 8)]
    for i, gr in enumerate([groups[0:3], groups[3:5], groups[5:7], groups[7:9]]):
        ffn(2 + i)
        for kas in gr:
            spectral(kas)

    ffn(6)
    butterflies(0, 64, 1)
    ffn(7)
    butterflies(64, 64, 1)

    rest[8].wait()
    outs = []
    for i in range(NB):
        rows = pl.ds(i * BM, BM)
        ye, yo = [_dot(jnp.concatenate([z_v[rows, pl.ds(p * 128, 128)], z_v[rows, pl.ds(H + p * 128, 128)]],
                                       axis=1).astype(BF16), gd_v[p]) for p in (0, 1)]
        y = jnp.concatenate([ye + yo, ye - yo], axis=1)
        o_v[rows, :] = (acc_v[rows, :] + y).astype(BF16)
        c = pltpu.make_async_copy(o_v.at[rows], o_h.at[rows], osem.at[i])
        c.start()
        outs.append(c)
    for c in outs:
        c.wait()


@jax.jit
def pallas_parallel_sum__spectral_gfnet__glu_gated_swiglu__prompt_kernel(
    A_x, A_w_r, A_w_i, B_x, B_w1, B_w3, B_w2,
):
    del B_x
    args = (A_x.reshape(S, D), A_w_r.T, A_w_i.T, B_w1.T, B_w3.T, B_w2) + _consts()
    out = pl.pallas_call(
        _kernel,
        out_shape=jax.ShapeDtypeStruct((S, D), BF16),
        in_specs=[pl.BlockSpec(memory_space=pltpu.MemorySpace.HBM)] * len(args),
        out_specs=pl.BlockSpec(memory_space=pl.ANY),
        scratch_shapes=[pltpu.VMEM(a.shape, a.dtype) for a in args] + [
            pltpu.VMEM((S, D), BF16), pltpu.VMEM((S, D), F32), pltpu.VMEM((S, D), F32),
            pltpu.VMEM((S, D), BF16), pltpu.VMEM((4, S, 128), F32),
            pltpu.SemaphoreType.DMA((16 + NB,)), pltpu.SemaphoreType.DMA((NB,))],
        compiler_params=pltpu.CompilerParams(vmem_limit_bytes=64 * 1024 * 1024),
    )(*args)
    return out.reshape(1, S, D)
```

```python
import math

import jax
import jax.numpy as jnp
import numpy as np
import jax.experimental.pallas as pl
import jax.experimental.pallas.tpu as pltpu

S, D, F = 2048, 512, 1376
R = 16
M = S // R
H = D // 2
BM = 256
NB = S // BM
BF16 = jnp.bfloat16
F32 = jnp.float32


def _consts():
    d = np.arange(D)[:, None]
    k = np.arange(H)[None, :]
    ang = 2 * np.pi * ((d * k) % D) / D
    fd = np.concatenate([np.cos(ang), -np.sin(ang)], axis=1)
    fd[:, H] = (-1.0) ** np.arange(D)
    gd = 2.0 * fd.T / D
    gd[0] /= 2
    gd[H] /= 2
    cols = [np.concatenate([np.arange(p, H, 2), H + np.arange(p, H, 2)]) for p in (0, 1)]
    fd = np.stack([fd[:H][:, c] for c in cols])
    gd = np.stack([gd[c][:, :H] for c in cols])
    b = np.arange(M)[None, :]
    kb = np.arange(M)[:, None]
    fs = []
    for ka in range(R):
        a = 2 * np.pi * ((b * (ka + R * kb)) % S) / S
        fr, fi = np.cos(a), -np.sin(a)
        fs.append(np.block([[fr, -fi], [fi, fr]]))
    fs = np.stack(fs)
    gs = np.transpose(fs, (0, 2, 1)) / S
    j = np.zeros((2, M, M))
    i = np.arange(M)
    j[0, i, (M - i) % M] = 1
    j[1, i, M - 1 - i] = 1
    c = lambda t: np.asarray(t, np.float32).astype(BF16)
    return c(fd), c(gd), c(fs), c(gs), c(j)


def _bf4(x, sign):
    (ar, ai), (br, bi), (cr, ci), (dr, di) = x
    sr, si, tr, ti = ar + cr, ai + ci, ar - cr, ai - ci
    ur, ui, vr, vi = br + dr, bi + di, br - dr, bi - di
    p = (tr + vi, ti - vr)
    q = (tr - vi, ti + vr)
    if sign > 0:
        p, q = q, p
    return [(sr + ur, si + ui), p, (sr - ur, si - ui), q]


def _tw(z, e, sign):
    r, i = z
    e = e % 16
    if e == 0:
        return z
    if e == 4:
        return (-i, r) if sign > 0 else (i, -r)
    c = math.cos(2 * math.pi * e / 16)
    s = sign * math.sin(2 * math.pi * e / 16)
    if e in (2, 6):
        if c * s > 0:
            return ((r - i) * c, (r + i) * c)
        return ((r + i) * c, (i - r) * c)
    return (r * c - i * s, i * c + r * s)


def _fft16(x, sign):
    t = [_bf4([x[4 * n1 + n2] for n1 in range(4)], sign) for n2 in range(4)]
    out = [None] * 16
    for k1 in range(4):
        o = _bf4([_tw(t[n2][k1], n2 * k1, sign) for n2 in range(4)], sign)
        for k2 in range(4):
            out[k1 + 4 * k2] = o[k2]
    return out


def _dot(a, b):
    return jnp.dot(a, b, preferred_element_type=F32)


def _dot_t(a, b):
    return jax.lax.dot_general(a, b, (((1,), (1,)), ((), ())), preferred_element_type=F32)


def _kernel(x_h, wr_h, wi_h, w1_h, w3_h, w2_h, fd_h, gd_h, fs_h, gs_h, j_h, o_h,
            x_v, wr_v, wi_v, w1_v, w3_v, w2_v, fd_v, gd_v, fs_v, gs_v, j_v,
            xn_v, z_v, acc_v, o_v, wu_v, sem, osem):
    cp = lambda s, d, i: pltpu.make_async_copy(s, d, sem.at[i])
    c_fd = cp(fd_h, fd_v, 0)
    c_x = [cp(x_h.at[pl.ds(i * BM, BM)], x_v.at[pl.ds(i * BM, BM)], 16 + i) for i in range(NB)]
    rest = [cp(w1_h, w1_v, 1), cp(w3_h, w3_v, 2), cp(w2_h, w2_v, 3), cp(fs_h, fs_v, 4),
            cp(wr_h, wr_v, 5), cp(wi_h, wi_v, 6), cp(j_h, j_v, 7), cp(gs_h, gs_v, 8),
            cp(gd_h, gd_v, 9)]
    c_x[0].start()
    c_fd.start()
    for c in c_x[1:3] + rest[:1]:
        c.start()

    c_fd.wait()
    for i in range(NB):
        c_x[i].wait()
        if i + 3 < NB:
            c_x[i + 3].start()
        if i == 4:
            rest[1].start()
        if i == 6:
            rest[2].start()
        rows = pl.ds(i * BM, BM)
        x = x_v[rows, :].astype(F32)
        xc = x - jnp.mean(x, axis=-1, keepdims=True)
        v = jnp.mean(xc * xc, axis=-1, keepdims=True)
        xn = (xc * jax.lax.rsqrt(v + 1e-5)).astype(BF16)
        xn_v[rows, :] = xn
        lo, hi = xn[:, :H].astype(F32), xn[:, H:].astype(F32)
        for p, t in enumerate((lo + hi, lo - hi)):
            t = _dot(t.astype(BF16), fd_v[p])
            z_v[rows, pl.ds(p * 128, 128)] = t[:, :128]
            z_v[rows, pl.ds(H + p * 128, 128)] = t[:, 128:]

    def ffn(i):
        if i % 2:
            return
        rows = pl.ds(i * BM, 2 * BM)
        xn = xn_v[rows, :]
        g = _dot_t(xn, w1_v[...])
        if i == 0:
            butterflies(0, 48, -1)
            rest[1].wait()
        u = _dot_t(xn, w3_v[...])
        h = (g * jax.nn.sigmoid(g) * u).astype(BF16)
        if i == 0:
            butterflies(48, 40, -1)
            rest[2].wait()
            for c in rest[6:]:
                c.start()
        acc_v[rows, :] = _dot(h, w2_v[...]) + x_v[rows, :].astype(F32)

    def butterflies(r0, n, sign):
        for r in range(n // 8):
            for c in range(H // 128):
                sl = lambda a, im: (pl.ds(a * M + r0 + 8 * r, 8), pl.ds(im * H + c * 128, 128))
                o = _fft16([(z_v[sl(a, 0)], z_v[sl(a, 1)]) for a in range(R)], sign)
                for a in range(R):
                    z_v[sl(a, 0)] = o[a][0]
                    z_v[sl(a, 1)] = o[a][1]

    def pack_w(i):
        for t in range(4):
            sl = pl.ds(i * 1024 + t * 256, 256)
            for n, ref in enumerate((wr_v, wi_v)):
                wu_v[n, sl, :] = pltpu.bitcast(ref[pl.ds(0, H), sl], F32).T
                wu_v[2 + n, sl, :] = jnp.broadcast_to(ref[pl.ds(H, 1), sl].astype(F32), (128, 256)).T

    def load_w(n, ka):
        w = wu_v[n, pl.ds(ka, M, stride=R), :]
        if n >= 2:
            return w
        u = jax.lax.bitcast_convert_type(w, jnp.uint32)
        return (jax.lax.bitcast_convert_type(u << 16, F32),
                jax.lax.bitcast_convert_type(u & jnp.uint32(0xFFFF0000), F32))

    lane0 = jax.lax.broadcasted_iota(jnp.int32, (M, 128), 1) == 0

    def spectral(kas):
        jm = j_v[0] if kas[0] == 0 else j_v[1]
        rev = lambda t: _dot(jm, t.astype(BF16))
        p, q, rm = {}, {}, {}
        for ka in kas:
            rows = pl.ds(ka * M, M)
            u = jnp.concatenate([z_v[rows, pl.ds(0, H)], z_v[rows, pl.ds(H, H)]], axis=0)
            t = _dot(fs_v[ka], u.astype(BF16))
            p[ka] = (t[:M], t[M:])
        for ka in kas:
            pr, pi = p[ka]
            (ur, ur1), (ui, ui1) = load_w(0, ka), load_w(1, ka)
            wr = jnp.concatenate([ur, ur1], axis=1)
            wi = jnp.concatenate([ui, ui1], axis=1)
            q[ka] = (pr * wr - pi * wi, pr * wi + pi * wr)
            vr, vi = load_w(2, ka), load_w(3, ka)
            nr, ni = p[(R - ka) % R]
            nr, ni = rev(nr[:, :128]), rev(ni[:, :128])
            pr, pi = pr[:, :128], pi[:, :128]
            ar, ai, br, bi = pr + nr, pi - ni, pr - nr, pi + ni
            er, ei = ar * ur - ai * ui, ar * ui + ai * ur
            fr, fi = br * vr - bi * vi, br * vi + bi * vr
            rm[ka] = (er + fr, ei + fi, er - fr, ei - fi)
        for ka in kas:
            qr, qi = q[ka]
            m = rm[(R - ka) % R]
            q0r = jnp.where(lane0, 0.25 * (rm[ka][0] + rev(m[2])), qr[:, :128])
            q0i = jnp.where(lane0, 0.25 * (rm[ka][1] - rev(m[3])), qi[:, :128])
            qq = jnp.concatenate([jnp.concatenate([q0r, qr[:, 128:]], axis=1),
                                  jnp.concatenate([q0i, qi[:, 128:]], axis=1)], axis=0)
            t = _dot(gs_v[ka], qq.astype(BF16))
            rows = pl.ds(ka * M, M)
            z_v[rows, pl.ds(0, H)] = t[:M]
            z_v[rows, pl.ds(H, H)] = t[M:]

    rest[0].wait()
    for c in rest[3:6]:
        c.start()
    ffn(0)
    butterflies(88, 40, -1)
    for c in rest[3:8]:
        c.wait()
    pack_w(0)
    pack_w(1)
    groups = [[0], [8]] + [[a, R - a] for a in range(1, 8)]
    for i, gr in enumerate([groups[0:3], groups[3:5], groups[5:7], groups[7:9]]):
        ffn(2 + i)
        for kas in gr:
            spectral(kas)

    ffn(6)
    butterflies(0, 64, 1)
    ffn(7)
    butterflies(64, 64, 1)

    rest[8].wait()
    outs = []
    for i in range(NB):
        rows = pl.ds(i * BM, BM)
        ye, yo = [_dot(jnp.concatenate([z_v[rows, pl.ds(p * 128, 128)], z_v[rows, pl.ds(H + p * 128, 128)]],
                                       axis=1).astype(BF16), gd_v[p]) for p in (0, 1)]
        y = jnp.concatenate([ye + yo, ye - yo], axis=1)
        o_v[rows, :] = (acc_v[rows, :] + y).astype(BF16)
        c = pltpu.make_async_copy(o_v.at[rows], o_h.at[rows], osem.at[i])
        c.start()
        outs.append(c)
    for c in outs:
        c.wait()


@jax.jit
def pallas_parallel_sum__spectral_gfnet__glu_gated_swiglu__prompt_kernel(
    A_x, A_w_r, A_w_i, B_x, B_w1, B_w3, B_w2,
):
    del B_x
    args = (A_x.reshape(S, D), A_w_r.T, A_w_i.T, B_w1.T, B_w3.T, B_w2) + _consts()
    out = pl.pallas_call(
        _kernel,
        out_shape=jax.ShapeDtypeStruct((S, D), BF16),
        in_specs=[pl.BlockSpec(memory_space=pltpu.MemorySpace.HBM)] * len(args),
        out_specs=pl.BlockSpec(memory_space=pl.ANY),
        scratch_shapes=[pltpu.VMEM(a.shape, a.dtype) for a in args] + [
            pltpu.VMEM((S, D), BF16), pltpu.VMEM((S, D), F32), pltpu.VMEM((S, D), F32),
            pltpu.VMEM((S, D), BF16), pltpu.VMEM((4, S, 128), F32),
            pltpu.SemaphoreType.DMA((16 + NB,)), pltpu.SemaphoreType.DMA((NB,))],
        compiler_params=pltpu.CompilerParams(vmem_limit_bytes=64 * 1024 * 1024),
    )(*args)
    return out.reshape(1, S, D)
```
